```python
import jax
import jax.numpy as jnp

def _softmax(x, axis=-1):
    return jax.nn.softmax(x, axis=axis)
def _gelu(x):
    return jax.nn.gelu(x, approximate=True)
def _silu(x):
    return jax.nn.silu(x)
def _sigmoid(x):
    return jax.nn.sigmoid(x)
def _layernorm(x, axis=-1, eps=1e-5):
    m = jnp.mean(x, axis=axis, keepdims=True)
    v = jnp.var(x, axis=axis, keepdims=True)
    return (x - m) / jnp.sqrt(v + eps)
def _scatter_add(tgt, idx, src, axis=0):
    return tgt.at[idx].add(src)
def _segment_sum(src, seg, n):
    return jax.ops.segment_sum(src, seg, n)
class _Rng:
    def __init__(self, key):
        self._k = key
    def _next(self):
        self._k, sub = jax.random.split(self._k)
        return sub
    def normal(self, shape):
        return jax.random.normal(self._next(), shape, dtype=jnp.bfloat16)
    def randint(self, lo, hi, shape):
        return jax.random.randint(self._next(), shape, lo, hi, dtype=jnp.int32)
    def uniform(self, shape, lo=0.0, hi=1.0):
        return jax.random.uniform(self._next(), shape, jnp.bfloat16, lo, hi)
    def permutation(self, n):
        return jax.random.permutation(self._next(), n)


kernel_name = 'interleave_layers__sliding_block_cached__dense_activation_gelu__decode'

def _fwd_setup_inputs():
    _rng = _Rng(jax.random.key(int.from_bytes(__import__("os").urandom(4), "little")))
    _w = (lambda a: (lambda t: t.astype(jnp.bfloat16) if jnp.issubdtype(t.dtype, jnp.floating) else t)(jnp.asarray(a)))
    def _A_setup():
        B, Sq, D = 2, 1, 512
        Hq, Hkv, Sk, Dh = 32, 8, 32768, 128
        assert Hq % Hkv == 0, (Hq, Hkv)
        return {
            "x": _w((lambda *s: _rng.normal(s) * 0.05)(B, Sq, D)),
            "k_cache": _w((lambda *s: _rng.normal(s) * 0.05)(B, Hkv, Sk, Dh)),
            "v_cache": _w((lambda *s: _rng.normal(s) * 0.05)(B, Hkv, Sk, Dh)),
            "wq": _w((lambda *s: _rng.normal(s) * 0.05)(D, Hq * Dh) * (D ** -0.5)),
            "wo": _w((lambda *s: _rng.normal(s) * 0.05)(Hq * Dh, D) * ((Hq * Dh) ** -0.5)),
        }
    _A_in = _A_setup()

    def _B_setup():
        B, S, D, F = 2, 1, 512, 1792
        return {
            "x": _w((lambda *s: _rng.normal(s) * 0.05)(B, S, D)),
            "w1": _w((lambda *s: _rng.normal(s) * 0.05)(D, F) * (D ** -0.5)),
            "b1": _w((lambda *s: _rng.normal(s) * 0.05)(F) * 0.01),
            "w2": _w((lambda *s: _rng.normal(s) * 0.05)(F, D) * (F ** -0.5)),
            "b2": _w((lambda *s: _rng.normal(s) * 0.05)(D) * 0.01),
        }
    _B_in = _B_setup()

    return {
        "A_x": _A_in["x"],
        "A_k_cache": _A_in["k_cache"],
        "A_v_cache": _A_in["v_cache"],
        "A_wq": _A_in["wq"],
        "A_wo": _A_in["wo"],
        "B_x": _B_in["x"],
        "B_w1": _B_in["w1"],
        "B_b1": _B_in["b1"],
        "B_w2": _B_in["w2"],
        "B_b2": _B_in["b2"],
    }

def _fwd_reference(A_x, A_k_cache, A_v_cache, A_wq, A_wo, B_x, B_w1, B_b1, B_w2, B_b2):
    def _A_ref(x, k_cache, v_cache, wq, wo):
        B, Sq, D = x.shape
        Hq, Dh = 32, 128
        Hkv, Sk = k_cache.shape[1], k_cache.shape[2]
        W = min(4096, max(256, Sk // 4))
        rep = Hq // Hkv
        q = (lambda x, *d: x.transpose(*d))((x @ wq).reshape(B, Sq, Hq, Dh), 0, 2, 1, 3)
        k = jnp.repeat(k_cache[:, :, Sk - W:, :], rep, axis=1)
        v = jnp.repeat(v_cache[:, :, Sk - W:, :], rep, axis=1)
        scores = jnp.einsum("bhqd,bhkd->bhqk", q, k) * (Dh ** -0.5)
        p = _softmax(scores, axis=-1)
        o = jnp.einsum("bhqk,bhkd->bhqd", p, v)
        return (lambda x, *d: x.transpose(*d))(o, 0, 2, 1, 3).reshape(B, Sq, Hq * Dh) @ wo

    def _B_ref(x, w1, b1, w2, b2):
        h = jnp.einsum("bsd,df->bsf", x, w1) + b1
        h = _gelu(h)
        return jnp.einsum("bsf,fd->bsd", h, w2) + b2

    x = A_x
    x = x + _A_ref(_layernorm(x, axis=-1), A_k_cache, A_v_cache, A_wq, A_wo)
    x = x + _B_ref(_layernorm(x, axis=-1), B_w1, B_b1, B_w2, B_b2)
    x = x + _A_ref(_layernorm(x, axis=-1), A_k_cache, A_v_cache, A_wq, A_wo)
    x = x + _B_ref(_layernorm(x, axis=-1), B_w1, B_b1, B_w2, B_b2)
    return x


def setup_inputs():
    _inp = _fwd_setup_inputs()
    _gk = jax.random.fold_in(jax.random.key(int.from_bytes(__import__("os").urandom(4), "little")), 2**31 - 1)
    _shapes = [[2, 1, 512]]
    _dtypes = ['bfloat16']
    _gks = jax.random.split(_gk, len(_shapes))
    _gs = [jax.random.normal(k, s, dtype=jnp.dtype(d)) * 0.05 for k, s, d in zip(_gks, _shapes, _dtypes)]
    _inp["grad_out"] = _gs[0]
    return _inp

def reference(A_x, A_k_cache, A_v_cache, A_wq, A_wo, B_w1, B_b1, B_w2, B_b2, B_x, grad_out):
    _const = dict(B_x=B_x)
    def _f(*_d):
        return _fwd_reference(**{'A_x': _d[0], 'A_k_cache': _d[1], 'A_v_cache': _d[2], 'A_wq': _d[3], 'A_wo': _d[4], 'B_w1': _d[5], 'B_b1': _d[6], 'B_w2': _d[7], 'B_b2': _d[8], **_const})
    _out, _vjp = jax.vjp(_f, A_x, A_k_cache, A_v_cache, A_wq, A_wo, B_w1, B_b1, B_w2, B_b2)
    _grads = _vjp(grad_out)
    _out0 = jnp.asarray(_out)
    return (_out0, *[jnp.asarray(_g) for _g in _grads])
```

```python
import math

import jax
import jax.numpy as jnp
from jax import lax
import jax.experimental.pallas as pl
import jax.experimental.pallas.tpu as pltpu

_EPS = 1e-5
_GELU_C = math.sqrt(2.0 / math.pi)
_GELU_A = 0.044715

_BF16 = jnp.bfloat16
_F32 = jnp.float32

_NN = (((1,), (0,)), ((), ()))
_NT = (((1,), (1,)), ((), ()))
_TN = (((0,), (0,)), ((), ()))


def _dot(a, b, dims):
    return lax.dot_general(
        a.astype(_BF16), b.astype(_BF16), dims, preferred_element_type=_F32
    )


def _ln_fwd(x):
    xc = x - jnp.mean(x, axis=-1, keepdims=True)
    rstd = lax.rsqrt(jnp.mean(xc * xc, axis=-1, keepdims=True) + _EPS)
    return xc * rstd, rstd


def _ln_bwd(dn, n, rstd):
    return rstd * (
        dn
        - jnp.mean(dn, axis=-1, keepdims=True)
        - n * jnp.mean(dn * n, axis=-1, keepdims=True)
    )


def _gelu_and_grad(h):
    h2 = h * h
    t = jnp.tanh(_GELU_C * (h + _GELU_A * h2 * h))
    cdf = 0.5 * (1.0 + t)
    return h * cdf, cdf + 0.5 * h * (1.0 - t * t) * (_GELU_C * (1.0 + 3.0 * _GELU_A * h2))


def _row(shape):
    return lax.broadcasted_iota(jnp.int32, shape, 0)


def _group_sum(z):
    r = _row(z.shape)
    z = z + jnp.where(r % 2 == 0, pltpu.roll(z, 7, 0), pltpu.roll(z, 1, 0))
    return z + jnp.where(r % 4 < 2, pltpu.roll(z, 6, 0), pltpu.roll(z, 2, 0))


def _replicate_rows(x2):
    n = x2.shape[1]
    return jnp.where(
        _row((8, n)) < 4,
        jnp.broadcast_to(x2[0:1], (8, n)),
        jnp.broadcast_to(x2[1:2], (8, n)),
    )


def _pick_batch_rows(x8):
    n = x8.shape[1]
    return jnp.where(
        _row((2, n)) == 0,
        jnp.broadcast_to(x8[0:1], (2, n)),
        jnp.broadcast_to(x8[4:5], (2, n)),
    )


def _start(copies):
    for i, c in enumerate(copies):
        c.start(priority=i % 2)


def _wait(copies):
    for c in copies:
        c.wait()


def _make_kernel(nb, hkv, rep, sk, win, dh, d, f):
    assert nb == 2 and rep == 4
    scale = dh ** -0.5
    gw = rep * dh
    zrows = 128
    rrows = 512
    n_zero = (sk - win) // zrows
    n_win = win // zrows
    key_chunk = 256

    z_first = 14
    z_step = 5
    assert z_first + 5 * hkv * z_step <= n_zero
    z_tail = n_zero - z_first - 5 * hkv * z_step

    def kernel(
        x_hbm, g_hbm, k_hbm, v_hbm, wq_hbm, wo_hbm, w1_hbm, b1_hbm, w2_hbm, b2_hbm,
        out_hbm, dx_hbm, dk_hbm, dv_hbm, dwq_hbm, dwo_hbm, dw1_hbm, db1_hbm, dw2_hbm,
        db2_hbm,
        x_s, g_s, b1_s, b2_s, k_s, v_s, wq_s, wo_s, w1_s, w2_s,
        out_s, dx_s, db1_s, db2_s, dk_s, dv_s, dwq_s, dwo_s, dw1_s, dw2_s,
        zero_s, q_s, do_s, p_s, ds_s, hm_s, sems,
    ):
        def row_chunks(src, dst, rows, sem):
            return [
                pltpu.make_async_copy(
                    src.at[pl.ds(r, rows), :], dst.at[pl.ds(r, rows), :], sem
                )
                for r in range(0, src.shape[0], rows)
            ]

        def cache_reads(bh):
            return [
                pltpu.make_async_copy(
                    src.at[bh, pl.ds(sk - win + r, rrows), :],
                    dst.at[bh, pl.ds(r, rrows), :],
                    sems.at[0],
                )
                for r in range(0, win, rrows)
                for src, dst in ((k_hbm, k_s), (v_hbm, v_s))
            ]

        @pl.loop(0, nb * hkv)
        def _(bh):
            _start(cache_reads(bh))

        small_reads = [
            pltpu.make_async_copy(src, dst, sems.at[1])
            for src, dst in ((x_hbm, x_s), (g_hbm, g_s), (b1_hbm, b1_s), (b2_hbm, b2_s))
        ]
        weight_reads = (
            row_chunks(wq_hbm, wq_s, 16, sems.at[1])
            + row_chunks(wo_hbm, wo_s, 128, sems.at[1])
            + row_chunks(w1_hbm, w1_s, 32, sems.at[1])
        )
        last_reads = row_chunks(w2_hbm, w2_s, 128, sems.at[2])
        _start(small_reads)
        _start(weight_reads)
        _start(last_reads)
        zero_s[...] = jnp.zeros(zero_s.shape, _BF16)

        @pl.loop(0, nb * hkv)
        def _(bh):
            _wait(cache_reads(bh))

        _wait(small_reads)
        _wait(weight_reads)

        def zero_writes(c):
            rows = pl.ds(pl.multiple_of(c * zrows, zrows), zrows)
            return [
                pltpu.make_async_copy(
                    zero_s, dst.at[pl.ds(b * hkv, hkv), rows, :], sems.at[3]
                )
                for b in range(nb)
                for dst in (dk_hbm, dv_hbm)
            ]

        def pump(first, count):
            @pl.loop(0, count)
            def _(i):
                _start(zero_writes(first + i))

        pump(0, z_first)
        _wait(last_reads)

        def pump_step(phase, h):
            pump(z_first + (phase * hkv + h) * z_step, z_step)

        row_d = _row((8, dh))

        def gather_heads(y, h_list=range(hkv)):
            res = []
            for h in h_list:
                t = y[:, h * gw : h * gw + dh]
                for g in range(1, rep):
                    t = jnp.where(
                        row_d % rep == g, y[:, h * gw + g * dh : h * gw + (g + 1) * dh], t
                    )
                res.append(t)
            return res

        def scatter_head(t):
            return jnp.concatenate(
                [jnp.where(row_d % rep == g, t, 0.0) for g in range(rep)], axis=1
            )

        def per_batch(a, ref, h, dims):
            r0 = _dot(a, ref[h], dims)
            r1 = _dot(a, ref[hkv + h], dims)
            return jnp.where(_row(r0.shape) < rep, r0, r1)

        def rows_of(layer):
            return pl.ds(8 * layer, 8)

        def attn_fwd(x, layer):
            n, rstd = _ln_fwd(x)
            for h, t in enumerate(gather_heads(_dot(n, wq_s[...], _NN))):
                q_s[h, rows_of(layer), :] = t

            @pl.loop(0, hkv)
            def _(h):
                pump_step(layer, h)
                s = per_batch(q_s[h, rows_of(layer), :], k_s, h, _NT) * scale
                e = jnp.exp(s - jnp.max(s, axis=-1, keepdims=True))
                p = e / jnp.sum(e, axis=-1, keepdims=True)
                p_s[h, rows_of(layer), :] = p
                hm_s[layer, h] = scatter_head(per_batch(p, v_s, h, _NN))

            o = jnp.concatenate([hm_s[layer, h] for h in range(hkv)], axis=1)
            return x + _group_sum(_dot(o, wo_s[...], _NN)), (n, rstd, o)

        def attn_bwd(dy, layer, n, rstd):
            for h, t in enumerate(gather_heads(_dot(dy, wo_s[...], _NT))):
                do_s[h, rows_of(layer), :] = t

            @pl.loop(0, hkv)
            def _(h):
                pump_step(3 - layer, h)
                p = p_s[h, rows_of(layer), :]
                dp = per_batch(do_s[h, rows_of(layer), :], v_s, h, _NT)
                ds = p * (dp - jnp.sum(p * dp, axis=-1, keepdims=True)) * scale
                ds_s[h, rows_of(layer), :] = ds
                hm_s[2 + layer, h] = scatter_head(per_batch(ds, k_s, h, _NN))

            dq = jnp.concatenate([hm_s[2 + layer, h] for h in range(hkv)], axis=1)
            dn = _group_sum(_dot(dq, wq_s[...], _NT))
            return dy + _ln_bwd(dn, n, rstd), dq

        b1 = b1_s[...].astype(_F32).reshape(1, f)
        b2 = b2_s[...].astype(_F32).reshape(1, d)

        def ffn_fwd(x):
            n, rstd = _ln_fwd(x)
            act, dact = _gelu_and_grad(_dot(n, w1_s[...], _NN) + b1)
            return x + _dot(act, w2_s[...], _NN) + b2, (n, rstd, act, dact)

        def ffn_bwd(dy, n, rstd, dact):
            dh_ = _dot(dy, w2_s[...], _NT) * dact
            return dy + _ln_bwd(_dot(dh_, w1_s[...], _NT), n, rstd), dh_

        x0 = _replicate_rows(x_s[...].astype(_F32))
        x1, (n0, r0, o0) = attn_fwd(x0, 0)
        x2, (n1, r1, a1, da1) = ffn_fwd(x1)
        x3, (n2, r2, o2) = attn_fwd(x2, 1)
        x4, (n3, r3, a3, da3) = ffn_fwd(x3)
        out_s[...] = _pick_batch_rows(x4).astype(_BF16)

        dx4 = _replicate_rows(g_s[...].astype(_F32))
        dx3, dh3 = ffn_bwd(dx4, n3, r3, da3)
        dx2, dq2 = attn_bwd(dx3, 1, n2, r2)
        dx1, dh1 = ffn_bwd(dx2, n1, r1, da1)
        dx0, dq0 = attn_bwd(dx1, 0, n0, r0)
        dx_s[...] = _pick_batch_rows(dx0).astype(_BF16)

        pump(z_first + 5 * hkv * z_step, z_tail)

        def layers(first, second):
            g = _row(first.shape) % rep
            return jnp.where(g == 0, first, jnp.where(g == 1, second, 0.0))

        def stack(first, second):
            return jnp.concatenate([first, second], axis=0)

        dh_l = layers(dh1, dh3)
        dy_l = layers(dx2, dx4)
        db1_s[...] = jnp.sum(dh_l, axis=0, keepdims=True).reshape(f).astype(_BF16)
        db2_s[...] = jnp.sum(dy_l, axis=0, keepdims=True).reshape(d).astype(_BF16)
        dw1_s[...] = _dot(layers(n1, n3), dh_l, _TN).astype(_BF16)
        dw2_s[...] = _dot(layers(a1, a3), dy_l, _TN).astype(_BF16)
        dwq_s[...] = _dot(stack(n0, n2), stack(dq0, dq2), _TN).astype(_BF16)
        dwo_s[...] = _dot(stack(o0, o2), stack(dx1, dx3), _TN).astype(_BF16)

        grad_writes = (
            [
                pltpu.make_async_copy(src, dst, sems.at[4])
                for src, dst in (
                    (out_s, out_hbm), (dx_s, dx_hbm), (db1_s, db1_hbm), (db2_s, db2_hbm)
                )
            ]
            + row_chunks(dwq_s, dwq_hbm, 16, sems.at[4])
            + row_chunks(dwo_s, dwo_hbm, 128, sems.at[4])
            + row_chunks(dw1_s, dw1_hbm, 32, sems.at[4])
            + row_chunks(dw2_s, dw2_hbm, 128, sems.at[4])
        )
        _start(grad_writes)

        def by_batch(t):
            b = (_row(t.shape) // rep) % nb
            return jnp.concatenate(
                [jnp.where(b == i, t, 0.0) for i in range(nb)], axis=1
            ).astype(_BF16)

        @pl.loop(0, hkv)
        def _(h):
            pump_step(4, h)
            for w_ref, t_ref, dst in ((ds_s, q_s, dk_s), (p_s, do_s, dv_s)):
                rhs = by_batch(t_ref[h])
                for c in range(0, win, key_chunk):
                    r = _dot(w_ref[h, :, c : c + key_chunk], rhs, _TN).astype(_BF16)
                    dst[h, c : c + key_chunk, :] = r[:, :dh]
                    dst[hkv + h, c : c + key_chunk, :] = r[:, dh:]

        def window_writes(c):
            r = pl.multiple_of(c * zrows, zrows)
            return [
                pltpu.make_async_copy(
                    src.at[pl.ds(b * hkv, hkv), pl.ds(r, zrows), :],
                    dst.at[pl.ds(b * hkv, hkv), pl.ds(sk - win + r, zrows), :],
                    sems.at[5],
                )
                for b in range(nb)
                for src, dst in ((dk_s, dk_hbm), (dv_s, dv_hbm))
            ]

        @pl.loop(0, n_win)
        def _(c):
            _start(window_writes(c))

        @pl.loop(0, n_zero)
        def _(c):
            _wait(zero_writes(c))

        _wait(grad_writes)

        @pl.loop(0, n_win)
        def _(c):
            _wait(window_writes(c))

    return kernel


@jax.jit
def pallas_interleave_layers__sliding_block_cached__dense_activation_gelu__decode_kernel(
    A_x: jax.Array,
    A_k_cache: jax.Array,
    A_v_cache: jax.Array,
    A_wq: jax.Array,
    A_wo: jax.Array,
    B_x: jax.Array,
    B_w1: jax.Array,
    B_b1: jax.Array,
    B_w2: jax.Array,
    B_b2: jax.Array,
    grad_out: jax.Array,
):
    del B_x
    nb, _, d = A_x.shape
    _, hkv, sk, dh = A_k_cache.shape
    rep = A_wq.shape[1] // (hkv * dh)
    f = B_w1.shape[1]
    win = min(4096, max(256, sk // 4))

    inputs = (
        A_x.reshape(nb, d), grad_out.reshape(nb, d),
        A_k_cache.reshape(nb * hkv, sk, dh), A_v_cache.reshape(nb * hkv, sk, dh),
        A_wq, A_wo, B_w1, B_b1, B_w2, B_b2,
    )
    out_shape = [
        jax.ShapeDtypeStruct(a.shape, _BF16) for a in (inputs[0],) + (inputs[0],) + inputs[2:]
    ]
    vmem = lambda *shape: pltpu.VMEM(shape, _BF16)
    vmem32 = lambda *shape: pltpu.VMEM(shape, _F32)
    staging = [
        vmem(nb, d), vmem(nb, d), vmem(f), vmem(d),
        vmem(nb * hkv, win, dh), vmem(nb * hkv, win, dh),
        vmem(*A_wq.shape), vmem(*A_wo.shape), vmem(*B_w1.shape), vmem(*B_w2.shape),
    ]
    hbm = pl.BlockSpec(memory_space=pltpu.HBM)

    out, dx, dk, dv, dwq, dwo, dw1, db1, dw2, db2 = pl.pallas_call(
        _make_kernel(nb, hkv, rep, sk, win, dh, d, f),
        out_shape=out_shape,
        in_specs=[hbm] * len(inputs),
        out_specs=[hbm] * len(out_shape),
        scratch_shapes=staging + staging + [
            vmem(hkv, 128, dh),
            vmem32(hkv, 16, dh), vmem32(hkv, 16, dh),
            vmem32(hkv, 16, win), vmem32(hkv, 16, win),
            vmem32(4, hkv, 8, rep * dh),
            pltpu.SemaphoreType.DMA((6,)),
        ],
        compiler_params=pltpu.CompilerParams(vmem_limit_bytes=112 * 1024 * 1024),
    )(*inputs)
    return (
        out.reshape(A_x.shape), dx.reshape(A_x.shape),
        dk.reshape(A_k_cache.shape), dv.reshape(A_v_cache.shape),
        dwq, dwo, dw1, db1, dw2, db2,
    )
```

```python
import math

import jax
import jax.numpy as jnp
from jax import lax
import jax.experimental.pallas as pl
import jax.experimental.pallas.tpu as pltpu

_EPS = 1e-5
_GELU_C = math.sqrt(2.0 / math.pi)
_GELU_A = 0.044715

_BF16 = jnp.bfloat16
_F32 = jnp.float32

_NN = (((1,), (0,)), ((), ()))
_NT = (((1,), (1,)), ((), ()))
_TN = (((0,), (0,)), ((), ()))

_STREAMS = 4
_READ_RUN = 32
_ZERO_RUN = 112
_WINDOW_RUN = 64

_ZERO_FIRST = 30
_ZERO_HEAD = 21
_ZERO_DENSE = 8

_KEY_CHUNK = 256


def _dot(a, b, dims):
    return lax.dot_general(
        a.astype(_BF16), b.astype(_BF16), dims, preferred_element_type=_F32
    )


def _ln_fwd(x):
    xc = x - jnp.mean(x, axis=-1, keepdims=True)
    rstd = lax.rsqrt(jnp.mean(xc * xc, axis=-1, keepdims=True) + _EPS)
    return xc * rstd, rstd


def _ln_bwd(dn, n, rstd):
    return rstd * (
        dn
        - jnp.mean(dn, axis=-1, keepdims=True)
        - n * jnp.mean(dn * n, axis=-1, keepdims=True)
    )


def _gelu_and_grad(h):
    h2 = h * h
    t = jnp.tanh(_GELU_C * (h + _GELU_A * h2 * h))
    cdf = 0.5 * (1.0 + t)
    du = _GELU_C * (1.0 + 3.0 * _GELU_A * h2)
    return h * cdf, cdf + 0.5 * h * (1.0 - t * t) * du


def _row(shape):
    return lax.broadcasted_iota(jnp.int32, shape, 0)


def _group_sum(z):
    r = _row(z.shape)
    z = z + jnp.where(r % 2 == 0, pltpu.roll(z, 7, 0), pltpu.roll(z, 1, 0))
    return z + jnp.where(r % 4 < 2, pltpu.roll(z, 6, 0), pltpu.roll(z, 2, 0))


def _replicate_rows(x2):
    n = x2.shape[1]
    return jnp.where(
        _row((8, n)) < 4,
        jnp.broadcast_to(x2[0:1], (8, n)),
        jnp.broadcast_to(x2[1:2], (8, n)),
    )


def _pick_batch_rows(x8):
    n = x8.shape[1]
    return jnp.where(
        _row((2, n)) == 0,
        jnp.broadcast_to(x8[0:1], (2, n)),
        jnp.broadcast_to(x8[4:5], (2, n)),
    )


def _by_layer(first, second):
    g = _row(first.shape) % 4
    return jnp.where(g == 0, first, jnp.where(g == 1, second, 0.0))


def _stack(first, second):
    return jnp.concatenate([first, second], axis=0)


def _matrix(ref):
    return ref[...].reshape(ref.shape[0] * ref.shape[1], ref.shape[2])


def _start(queues):
    for i in range(max(len(q) for q in queues)):
        for priority, q in enumerate(queues):
            if i < len(q):
                q[i].start(priority=priority)


def _wait(queues):
    for q in queues:
        for copy in q:
            copy.wait()


def _tile_copy(src, dst, sem, lead, rows, cols):
    return pltpu.make_async_copy(src.at[lead, rows, cols], dst.at[lead, rows, cols], sem)


def _make_kernel(nb, hkv, rep, sk, win, dh, d, f):
    assert nb == 2 and rep == 4
    scale = dh ** -0.5
    gw = rep * dh
    n_groups = nb * hkv // _STREAMS
    zero_runs = (sk - win) // _ZERO_RUN
    window_runs = win // _WINDOW_RUN
    assert zero_runs * _ZERO_RUN == sk - win
    n_zero = n_groups * zero_runs
    n_window = n_groups * window_runs
    assert n_zero % n_window == 0
    read_unroll = 16
    read_steps = win // (_READ_RUN * read_unroll)
    attn_steps = d // _STREAMS // 8
    ffn_steps = d // _STREAMS // 16
    ffn_late = 2
    w2_rows = f // _STREAMS // ffn_steps
    assert w2_rows % 8 == 0 and w2_rows * ffn_steps * _STREAMS == f

    def kernel(
        x_hbm, g_hbm, k_hbm, v_hbm, wq_hbm, wo_hbm, w1_hbm, b1_hbm, w2_hbm, b2_hbm,
        out_hbm, dx_hbm, dk_hbm, dv_hbm, dwq_hbm, dwo_hbm, dw1_hbm, db1_hbm, dw2_hbm,
        db2_hbm,
        x_s, g_s, k_s, v_s, wq_s, wo_s, w1_s, b1_s, w2_s, b2_s,
        out_s, dx_s, dk_s, dv_s, dwq_s, dwo_s, dw1_s, db1_s, dw2_s, db2_s,
        zero_s, q_s, do_s, p_s, ds_s, feat_s, sems,
    ):
        early_sem, late_sem, zero_sem, grad_sem, window_sem = (
            sems.at[i] for i in range(5)
        )
        every = slice(None)

        def cache_reads(i):
            group = i // read_steps
            heads = pl.ds(group * _STREAMS, _STREAMS)
            base = pl.multiple_of(
                (i - group * read_steps) * (_READ_RUN * read_unroll), _READ_RUN
            )
            return [
                [
                    pltpu.make_async_copy(
                        src.at[heads, pl.ds(sk - win + base + u * _READ_RUN, _READ_RUN), :],
                        dst.at[heads, pl.ds(base + u * _READ_RUN, _READ_RUN), :],
                        early_sem,
                    )
                    for u in range(read_unroll)
                ]
                for src, dst in ((k_hbm, k_s), (v_hbm, v_s))
            ]

        def small_reads():
            return [
                [pltpu.make_async_copy(src, dst, early_sem) for src, dst in q]
                for q in (((x_hbm, x_s), (b1_hbm, b1_s)), ((g_hbm, g_s), (b2_hbm, b2_s)))
            ]

        def attn_weight_reads(i):
            wq_rows = pl.ds(pl.multiple_of(i * 8, 8), 8)
            return [
                [
                    _tile_copy(wq_hbm, wq_s, early_sem, every, wq_rows, pl.ds(h * gw, gw))
                    for h in range(hkv)
                ],
                [
                    _tile_copy(
                        wo_hbm, wo_s, early_sem, every,
                        pl.ds(pl.multiple_of((i * hkv + h) * 8, 8), 8), every,
                    )
                    for h in range(hkv)
                ],
            ]

        def ffn_weight_reads(i, sem):
            return [
                [
                    _tile_copy(
                        w1_hbm, w1_s, sem, pl.ds(lead, 2),
                        pl.ds(pl.multiple_of(i * 16 + r, 8), 8), pl.ds(c, f // 2),
                    )
                    for r in (0, 8)
                    for c in (0, f // 2)
                    for lead in range(0, _STREAMS, 2)
                ],
                [
                    _tile_copy(
                        w2_hbm, w2_s, sem, every,
                        pl.ds(pl.multiple_of(i * w2_rows + r, 8), 8), every,
                    )
                    for r in range(0, w2_rows, 8)
                ],
            ]

        def early_reads(action):
            pl.loop(0, n_groups * read_steps)(lambda i: action(cache_reads(i)))
            action(small_reads())
            pl.loop(0, attn_steps)(lambda i: action(attn_weight_reads(i)))
            pl.loop(0, ffn_steps - ffn_late)(
                lambda i: action(ffn_weight_reads(i, early_sem))
            )

        def late_reads(action):
            pl.loop(ffn_steps - ffn_late, ffn_steps)(
                lambda i: action(ffn_weight_reads(i, late_sem))
            )

        early_reads(_start)
        late_reads(_start)
        zero_s[...] = jnp.zeros(zero_s.shape, _BF16)
        early_reads(_wait)

        def zero_writes(i):
            group = i // zero_runs
            heads = pl.ds(group * _STREAMS, _STREAMS)
            rows = pl.ds(
                pl.multiple_of((i - group * zero_runs) * _ZERO_RUN, 16), _ZERO_RUN
            )
            return [
                [pltpu.make_async_copy(zero_s, dst.at[heads, rows, :], zero_sem)]
                for dst in (dk_hbm, dv_hbm)
            ]

        zeros_issued = [0]

        def reserve_zeros(count):
            first = zeros_issued[0]
            zeros_issued[0] += count
            assert zeros_issued[0] <= n_zero
            return first

        def start_zeros(first, count):
            pl.loop(0, count)(lambda i: _start(zero_writes(first + i)))

        def more_zeros(count=_ZERO_DENSE):
            start_zeros(reserve_zeros(count), count)

        def for_each_head(body):
            first = reserve_zeros(hkv * _ZERO_HEAD)

            @pl.loop(0, hkv)
            def _(h):
                start_zeros(first + h * _ZERO_HEAD, _ZERO_HEAD)
                body(h)

        more_zeros(_ZERO_FIRST)
        late_reads(_wait)

        slot = _row((8, dh)) % rep

        def rows_of(layer):
            return pl.ds(8 * layer, 8)

        def gather_heads(y, dst, layer):
            for h in range(hkv):
                t = y[:, h * gw : h * gw + dh]
                for g in range(1, rep):
                    t = jnp.where(slot == g, y[:, h * gw + g * dh : h * gw + (g + 1) * dh], t)
                dst[h, rows_of(layer), :] = t

        def scatter_head(t):
            return jnp.concatenate(
                [jnp.where(slot == g, t, 0.0) for g in range(rep)], axis=1
            )

        def per_batch(a, cache, h, dims):
            r0 = _dot(a, cache[h], dims)
            r1 = _dot(a, cache[hkv + h], dims)
            return jnp.where(_row(r0.shape) < rep, r0, r1)

        def all_heads(i):
            return jnp.concatenate([feat_s[i, h] for h in range(hkv)], axis=1)

        def attn_fwd(x, layer):
            more_zeros()
            n, rstd = _ln_fwd(x)
            gather_heads(_dot(n, _matrix(wq_s), _NN), q_s, layer)

            @for_each_head
            def _(h):
                s = per_batch(q_s[h, rows_of(layer), :], k_s, h, _NT) * scale
                e = jnp.exp(s - jnp.max(s, axis=-1, keepdims=True))
                p = e / jnp.sum(e, axis=-1, keepdims=True)
                p_s[h, rows_of(layer), :] = p
                feat_s[layer, h] = scatter_head(per_batch(p, v_s, h, _NN))

            more_zeros()
            o = all_heads(layer)
            return x + _group_sum(_dot(o, _matrix(wo_s), _NN)), (n, rstd, o)

        def attn_bwd(dy, layer, n, rstd):
            more_zeros()
            gather_heads(_dot(dy, _matrix(wo_s), _NT), do_s, layer)

            @for_each_head
            def _(h):
                p = p_s[h, rows_of(layer), :]
                dp = per_batch(do_s[h, rows_of(layer), :], v_s, h, _NT)
                ds = p * (dp - jnp.sum(p * dp, axis=-1, keepdims=True)) * scale
                ds_s[h, rows_of(layer), :] = ds
                feat_s[2 + layer, h] = scatter_head(per_batch(ds, k_s, h, _NN))

            more_zeros()
            dq = all_heads(2 + layer)
            dn = _group_sum(_dot(dq, _matrix(wq_s), _NT))
            return dy + _ln_bwd(dn, n, rstd), dq

        b1 = b1_s[...].astype(_F32).reshape(1, f)
        b2 = b2_s[...].astype(_F32).reshape(1, d)

        def ffn_fwd(x):
            more_zeros()
            n, rstd = _ln_fwd(x)
            act, dact = _gelu_and_grad(_dot(n, _matrix(w1_s), _NN) + b1)
            return x + _dot(act, _matrix(w2_s), _NN) + b2, (n, rstd, act, dact)

        def ffn_bwd(dy, n, rstd, dact):
            more_zeros()
            dpre = _dot(dy, _matrix(w2_s), _NT) * dact
            return dy + _ln_bwd(_dot(dpre, _matrix(w1_s), _NT), n, rstd), dpre

        x0 = _replicate_rows(x_s[...].astype(_F32))
        x1, (n0, r0, o0) = attn_fwd(x0, 0)
        x2, (n1, r1, a1, da1) = ffn_fwd(x1)
        x3, (n2, r2, o2) = attn_fwd(x2, 1)
        x4, (n3, r3, a3, da3) = ffn_fwd(x3)
        out_s[...] = _pick_batch_rows(x4).astype(_BF16)

        dx4 = _replicate_rows(g_s[...].astype(_F32))
        dx3, dpre3 = ffn_bwd(dx4, n3, r3, da3)
        dx2, dq2 = attn_bwd(dx3, 1, n2, r2)
        dx1, dpre1 = ffn_bwd(dx2, n1, r1, da1)
        dx0, dq0 = attn_bwd(dx1, 0, n0, r0)
        dx_s[...] = _pick_batch_rows(dx0).astype(_BF16)

        def weight_grad(dst, a, b):
            more_zeros()
            rows = dst.shape[1]
            for i in range(_STREAMS):
                dst[i] = _dot(a[:, i * rows : (i + 1) * rows], b, _TN).astype(_BF16)

        dpre = _by_layer(dpre1, dpre3)
        dffn = _by_layer(dx2, dx4)
        db1_s[...] = jnp.sum(dpre, axis=0, keepdims=True).reshape(f).astype(_BF16)
        db2_s[...] = jnp.sum(dffn, axis=0, keepdims=True).reshape(d).astype(_BF16)
        weight_grad(dw1_s, _by_layer(n1, n3), dpre)
        weight_grad(dw2_s, _by_layer(a1, a3), dffn)
        weight_grad(dwq_s, _stack(n0, n2), _stack(dq0, dq2))
        weight_grad(dwo_s, _stack(o0, o2), _stack(dx1, dx3))

        def weight_writes(src, dst):
            _, rows, cols = src.shape
            c = min(cols, 2048)
            r = max(8, 16384 // c // 8 * 8)
            return [
                _tile_copy(src, dst, grad_sem, every, pl.ds(i, r), pl.ds(j, c))
                for i in range(0, rows, r)
                for j in range(0, cols, c)
            ]

        def grad_writes():
            whole = lambda src, dst: pltpu.make_async_copy(src, dst, grad_sem)
            return [
                [whole(out_s, out_hbm), whole(db1_s, db1_hbm)]
                + weight_writes(dwq_s, dwq_hbm)
                + weight_writes(dw1_s, dw1_hbm),
                [whole(dx_s, dx_hbm), whole(db2_s, db2_hbm)]
                + weight_writes(dwo_s, dwo_hbm)
                + weight_writes(dw2_s, dw2_hbm),
            ]

        _start(grad_writes())

        def by_batch(t):
            b = (_row(t.shape) // rep) % nb
            return jnp.concatenate(
                [jnp.where(b == i, t, 0.0) for i in range(nb)], axis=1
            ).astype(_BF16)

        @for_each_head
        def _(h):
            for key_ref, feat_ref, dst in ((ds_s, q_s, dk_s), (p_s, do_s, dv_s)):
                rhs = by_batch(feat_ref[h])
                for c in range(0, win, _KEY_CHUNK):
                    keys = slice(c, c + _KEY_CHUNK)
                    r = _dot(key_ref[h, :, keys], rhs, _TN).astype(_BF16)
                    dst[h, keys, :] = r[:, :dh]
                    dst[hkv + h, keys, :] = r[:, dh:]

        more_zeros(n_zero - zeros_issued[0])

        def window_writes(i):
            group = i // window_runs
            heads = pl.ds(group * _STREAMS, _STREAMS)
            r = pl.multiple_of((i - group * window_runs) * _WINDOW_RUN, _WINDOW_RUN)
            return [
                [
                    pltpu.make_async_copy(
                        src.at[heads, pl.ds(r, _WINDOW_RUN), :],
                        dst.at[heads, pl.ds(sk - win + r, _WINDOW_RUN), :],
                        window_sem,
                    )
                ]
                for src, dst in ((dk_s, dk_hbm), (dv_s, dv_hbm))
            ]

        zeros_per_window = n_zero // n_window

        @pl.loop(0, n_window)
        def _(i):
            _start(window_writes(i))
            for j in range(zeros_per_window):
                _wait(zero_writes(i * zeros_per_window + j))

        _wait(grad_writes())
        pl.loop(0, n_window)(lambda i: _wait(window_writes(i)))

    return kernel


@jax.jit
def pallas_interleave_layers__sliding_block_cached__dense_activation_gelu__decode_kernel(
    A_x: jax.Array,
    A_k_cache: jax.Array,
    A_v_cache: jax.Array,
    A_wq: jax.Array,
    A_wo: jax.Array,
    B_x: jax.Array,
    B_w1: jax.Array,
    B_b1: jax.Array,
    B_w2: jax.Array,
    B_b2: jax.Array,
    grad_out: jax.Array,
):
    del B_x
    nb, _, d = A_x.shape
    _, hkv, sk, dh = A_k_cache.shape
    rep = A_wq.shape[1] // (hkv * dh)
    f = B_w1.shape[1]
    win = min(4096, max(256, sk // 4))
    assert rep * dh == d

    def split_rows(w):
        return w.reshape(_STREAMS, w.shape[0] // _STREAMS, w.shape[1])

    inputs = (
        A_x.reshape(nb, d),
        grad_out.reshape(nb, d),
        A_k_cache.reshape(nb * hkv, sk, dh),
        A_v_cache.reshape(nb * hkv, sk, dh),
        split_rows(A_wq),
        split_rows(A_wo),
        split_rows(B_w1),
        B_b1,
        split_rows(B_w2),
        B_b2,
    )
    out_shape = [jax.ShapeDtypeStruct(a.shape, _BF16) for a in inputs]
    staging = [pltpu.VMEM(a.shape, _BF16) for a in inputs]
    staging[2] = staging[3] = pltpu.VMEM((nb * hkv, win, dh), _BF16)
    hbm = pl.BlockSpec(memory_space=pltpu.HBM)

    out, dx, dk, dv, dwq, dwo, dw1, db1, dw2, db2 = pl.pallas_call(
        _make_kernel(nb, hkv, rep, sk, win, dh, d, f),
        out_shape=out_shape,
        in_specs=[hbm] * len(inputs),
        out_specs=[hbm] * len(out_shape),
        scratch_shapes=staging + staging + [
            pltpu.VMEM((_STREAMS, _ZERO_RUN, dh), _BF16),
            pltpu.VMEM((hkv, 16, dh), _F32),
            pltpu.VMEM((hkv, 16, dh), _F32),
            pltpu.VMEM((hkv, 16, win), _F32),
            pltpu.VMEM((hkv, 16, win), _F32),
            pltpu.VMEM((4, hkv, 8, rep * dh), _F32),
            pltpu.SemaphoreType.DMA((5,)),
        ],
        compiler_params=pltpu.CompilerParams(vmem_limit_bytes=112 * 1024 * 1024),
    )(*inputs)
    return (
        out.reshape(A_x.shape),
        dx.reshape(A_x.shape),
        dk.reshape(A_k_cache.shape),
        dv.reshape(A_v_cache.shape),
        dwq.reshape(A_wq.shape),
        dwo.reshape(A_wo.shape),
        dw1.reshape(B_w1.shape),
        db1,
        dw2.reshape(B_w2.shape),
        db2,
    )
```

```python
import math

import jax
import jax.numpy as jnp
from jax import lax
import jax.experimental.pallas as pl
import jax.experimental.pallas.tpu as pltpu

_EPS = 1e-5
_GELU_C = math.sqrt(2.0 / math.pi)
_GELU_A = 0.044715

_BF16 = jnp.bfloat16
_F32 = jnp.float32

_NN = (((1,), (0,)), ((), ()))
_NT = (((1,), (1,)), ((), ()))
_TN = (((0,), (0,)), ((), ()))

_STREAMS = 4
_READ_RUN = 32
_ZERO_RUN = 112
_ZERO_STAGGER = 6
_WINDOW_RUN = 64

_ZERO_FIRST = 30
_ZERO_HEAD = 21
_ZERO_DENSE = 8

_KEY_CHUNK = 256


def _dot(a, b, dims):
    return lax.dot_general(
        a.astype(_BF16), b.astype(_BF16), dims, preferred_element_type=_F32
    )


def _ln_fwd(x):
    xc = x - jnp.mean(x, axis=-1, keepdims=True)
    rstd = lax.rsqrt(jnp.mean(xc * xc, axis=-1, keepdims=True) + _EPS)
    return xc * rstd, rstd


def _ln_bwd(dn, n, rstd):
    return rstd * (
        dn
        - jnp.mean(dn, axis=-1, keepdims=True)
        - n * jnp.mean(dn * n, axis=-1, keepdims=True)
    )


def _gelu_and_grad(h):
    h2 = h * h
    t = jnp.tanh(_GELU_C * (h + _GELU_A * h2 * h))
    cdf = 0.5 * (1.0 + t)
    du = _GELU_C * (1.0 + 3.0 * _GELU_A * h2)
    return h * cdf, cdf + 0.5 * h * (1.0 - t * t) * du


def _row(shape):
    return lax.broadcasted_iota(jnp.int32, shape, 0)


def _group_sum(z):
    r = _row(z.shape)
    z = z + jnp.where(r % 2 == 0, pltpu.roll(z, 7, 0), pltpu.roll(z, 1, 0))
    return z + jnp.where(r % 4 < 2, pltpu.roll(z, 6, 0), pltpu.roll(z, 2, 0))


def _replicate_rows(x2):
    n = x2.shape[1]
    return jnp.where(
        _row((8, n)) < 4,
        jnp.broadcast_to(x2[0:1], (8, n)),
        jnp.broadcast_to(x2[1:2], (8, n)),
    )


def _pick_batch_rows(x8):
    n = x8.shape[1]
    return jnp.where(
        _row((2, n)) == 0,
        jnp.broadcast_to(x8[0:1], (2, n)),
        jnp.broadcast_to(x8[4:5], (2, n)),
    )


def _by_layer(first, second):
    g = _row(first.shape) % 4
    return jnp.where(g == 0, first, jnp.where(g == 1, second, 0.0))


def _stack(first, second):
    return jnp.concatenate([first, second], axis=0)


def _matrix(ref):
    return ref[...].reshape(ref.shape[0] * ref.shape[1], ref.shape[2])


def _start(queues):
    for i in range(max(len(q) for q in queues)):
        for priority, q in enumerate(queues):
            if i < len(q):
                q[i].start(priority=priority)


def _wait(queues):
    for q in queues:
        for copy in q:
            copy.wait()


def _tile_copy(src, dst, sem, lead, rows, cols):
    return pltpu.make_async_copy(src.at[lead, rows, cols], dst.at[lead, rows, cols], sem)


def _make_kernel(nb, hkv, rep, sk, win, dh, d, f):
    assert nb == 2 and rep == 4
    scale = dh ** -0.5
    gw = rep * dh
    n_groups = nb * hkv // _STREAMS
    zero_runs = (sk - win) // _ZERO_RUN
    window_runs = win // _WINDOW_RUN
    assert zero_runs * _ZERO_RUN == sk - win
    n_zero = n_groups * zero_runs
    n_window = n_groups * window_runs
    assert n_zero % n_window == 0
    read_unroll = 16
    read_steps = win // (_READ_RUN * read_unroll)
    attn_steps = d // _STREAMS // 8
    ffn_steps = d // _STREAMS // 16
    ffn_late = 2
    w2_rows = f // _STREAMS // ffn_steps
    assert w2_rows % 8 == 0 and w2_rows * ffn_steps * _STREAMS == f

    def kernel(
        x_hbm, g_hbm, k_hbm, v_hbm, wq_hbm, wo_hbm, w1_hbm, b1_hbm, w2_hbm, b2_hbm,
        out_hbm, dx_hbm, dk_hbm, dv_hbm, dwq_hbm, dwo_hbm, dw1_hbm, db1_hbm, dw2_hbm,
        db2_hbm,
        x_s, g_s, k_s, v_s, wq_s, wo_s, w1_s, b1_s, w2_s, b2_s,
        out_s, dx_s, dk_s, dv_s, dwq_s, dwo_s, dw1_s, db1_s, dw2_s, db2_s,
        zero_s, q_s, do_s, p_s, ds_s, feat_s, sems,
    ):
        early_sem, late_sem, zero_sem, grad_sem, window_sem = (
            sems.at[i] for i in range(5)
        )
        every = slice(None)

        def cache_reads(i):
            group = i // read_steps
            heads = pl.ds(group * _STREAMS, _STREAMS)
            base = pl.multiple_of(
                (i - group * read_steps) * (_READ_RUN * read_unroll), _READ_RUN
            )
            return [
                [
                    pltpu.make_async_copy(
                        src.at[heads, pl.ds(sk - win + base + u * _READ_RUN, _READ_RUN), :],
                        dst.at[heads, pl.ds(base + u * _READ_RUN, _READ_RUN), :],
                        early_sem,
                    )
                    for u in range(read_unroll)
                ]
                for src, dst in ((k_hbm, k_s), (v_hbm, v_s))
            ]

        def small_reads():
            return [
                [pltpu.make_async_copy(src, dst, early_sem) for src, dst in q]
                for q in (((x_hbm, x_s), (b1_hbm, b1_s)), ((g_hbm, g_s), (b2_hbm, b2_s)))
            ]

        def attn_weight_reads(i):
            wq_rows = pl.ds(pl.multiple_of(i * 8, 8), 8)
            return [
                [
                    _tile_copy(wq_hbm, wq_s, early_sem, every, wq_rows, pl.ds(h * gw, gw))
                    for h in range(hkv)
                ],
                [
                    _tile_copy(
                        wo_hbm, wo_s, early_sem, every,
                        pl.ds(pl.multiple_of((i * hkv + h) * 8, 8), 8), every,
                    )
                    for h in range(hkv)
                ],
            ]

        def ffn_weight_reads(i, sem):
            return [
                [
                    _tile_copy(
                        w1_hbm, w1_s, sem, pl.ds(lead, 2),
                        pl.ds(pl.multiple_of(i * 16 + r, 8), 8), pl.ds(c, f // 2),
                    )
                    for r in (0, 8)
                    for c in (0, f // 2)
                    for lead in range(0, _STREAMS, 2)
                ],
                [
                    _tile_copy(
                        w2_hbm, w2_s, sem, every,
                        pl.ds(pl.multiple_of(i * w2_rows + r, 8), 8), every,
                    )
                    for r in range(0, w2_rows, 8)
                ],
            ]

        def early_reads(action):
            pl.loop(0, n_groups * read_steps)(lambda i: action(cache_reads(i)))
            action(small_reads())
            pl.loop(0, attn_steps)(lambda i: action(attn_weight_reads(i)))
            pl.loop(0, ffn_steps - ffn_late)(
                lambda i: action(ffn_weight_reads(i, early_sem))
            )

        def late_reads(action):
            pl.loop(ffn_steps - ffn_late, ffn_steps)(
                lambda i: action(ffn_weight_reads(i, late_sem))
            )

        early_reads(_start)
        late_reads(_start)
        zero_s[...] = jnp.zeros(zero_s.shape, _BF16)
        early_reads(_wait)

        def zero_writes(i):
            group = i // zero_runs
            heads = pl.ds(group * _STREAMS, _STREAMS)
            run = i - group * zero_runs
            return [
                [
                    pltpu.make_async_copy(
                        zero_s,
                        dst.at[heads, pl.ds(pl.multiple_of(r * _ZERO_RUN, 16), _ZERO_RUN), :],
                        zero_sem,
                    )
                ]
                for dst, r in ((dk_hbm, run), (dv_hbm, (run + _ZERO_STAGGER) % zero_runs))
            ]

        zeros_issued = [0]

        def reserve_zeros(count):
            first = zeros_issued[0]
            zeros_issued[0] += count
            assert zeros_issued[0] <= n_zero
            return first

        def start_zeros(first, count):
            pl.loop(0, count)(lambda i: _start(zero_writes(first + i)))

        def more_zeros(count=_ZERO_DENSE):
            start_zeros(reserve_zeros(count), count)

        def for_each_head(body):
            first = reserve_zeros(hkv * _ZERO_HEAD)

            @pl.loop(0, hkv)
            def _(h):
                start_zeros(first + h * _ZERO_HEAD, _ZERO_HEAD)
                body(h)

        more_zeros(_ZERO_FIRST)
        late_reads(_wait)

        slot = _row((8, dh)) % rep

        def rows_of(layer):
            return pl.ds(8 * layer, 8)

        def gather_heads(y, dst, layer):
            for h in range(hkv):
                t = y[:, h * gw : h * gw + dh]
                for g in range(1, rep):
                    t = jnp.where(slot == g, y[:, h * gw + g * dh : h * gw + (g + 1) * dh], t)
                dst[h, rows_of(layer), :] = t

        def scatter_head(t):
            return jnp.concatenate(
                [jnp.where(slot == g, t, 0.0) for g in range(rep)], axis=1
            )

        def per_batch(a, cache, h, dims):
            r0 = _dot(a, cache[h], dims)
            r1 = _dot(a, cache[hkv + h], dims)
            return jnp.where(_row(r0.shape) < rep, r0, r1)

        def all_heads(i):
            return jnp.concatenate([feat_s[i, h] for h in range(hkv)], axis=1)

        def attn_fwd(x, layer):
            more_zeros()
            n, rstd = _ln_fwd(x)
            gather_heads(_dot(n, _matrix(wq_s), _NN), q_s, layer)

            @for_each_head
            def _(h):
                s = per_batch(q_s[h, rows_of(layer), :], k_s, h, _NT) * scale
                e = jnp.exp(s - jnp.max(s, axis=-1, keepdims=True))
                p = e / jnp.sum(e, axis=-1, keepdims=True)
                p_s[h, rows_of(layer), :] = p
                feat_s[layer, h] = scatter_head(per_batch(p, v_s, h, _NN))

            more_zeros()
            o = all_heads(layer)
            return x + _group_sum(_dot(o, _matrix(wo_s), _NN)), (n, rstd, o)

        def attn_bwd(dy, layer, n, rstd):
            more_zeros()
            gather_heads(_dot(dy, _matrix(wo_s), _NT), do_s, layer)

            @for_each_head
            def _(h):
                p = p_s[h, rows_of(layer), :]
                dp = per_batch(do_s[h, rows_of(layer), :], v_s, h, _NT)
                ds = p * (dp - jnp.sum(p * dp, axis=-1, keepdims=True)) * scale
                ds_s[h, rows_of(layer), :] = ds
                feat_s[2 + layer, h] = scatter_head(per_batch(ds, k_s, h, _NN))

            more_zeros()
            dq = all_heads(2 + layer)
            dn = _group_sum(_dot(dq, _matrix(wq_s), _NT))
            return dy + _ln_bwd(dn, n, rstd), dq

        b1 = b1_s[...].astype(_F32).reshape(1, f)
        b2 = b2_s[...].astype(_F32).reshape(1, d)

        def ffn_fwd(x):
            more_zeros()
            n, rstd = _ln_fwd(x)
            act, dact = _gelu_and_grad(_dot(n, _matrix(w1_s), _NN) + b1)
            return x + _dot(act, _matrix(w2_s), _NN) + b2, (n, rstd, act, dact)

        def ffn_bwd(dy, n, rstd, dact):
            more_zeros()
            dpre = _dot(dy, _matrix(w2_s), _NT) * dact
            return dy + _ln_bwd(_dot(dpre, _matrix(w1_s), _NT), n, rstd), dpre

        x0 = _replicate_rows(x_s[...].astype(_F32))
        x1, (n0, r0, o0) = attn_fwd(x0, 0)
        x2, (n1, r1, a1, da1) = ffn_fwd(x1)
        x3, (n2, r2, o2) = attn_fwd(x2, 1)
        x4, (n3, r3, a3, da3) = ffn_fwd(x3)
        out_s[...] = _pick_batch_rows(x4).astype(_BF16)

        dx4 = _replicate_rows(g_s[...].astype(_F32))
        dx3, dpre3 = ffn_bwd(dx4, n3, r3, da3)
        dx2, dq2 = attn_bwd(dx3, 1, n2, r2)
        dx1, dpre1 = ffn_bwd(dx2, n1, r1, da1)
        dx0, dq0 = attn_bwd(dx1, 0, n0, r0)
        dx_s[...] = _pick_batch_rows(dx0).astype(_BF16)

        def weight_grad(dst, a, b):
            more_zeros()
            rows = dst.shape[1]
            for i in range(_STREAMS):
                dst[i] = _dot(a[:, i * rows : (i + 1) * rows], b, _TN).astype(_BF16)

        dpre = _by_layer(dpre1, dpre3)
        dffn = _by_layer(dx2, dx4)
        db1_s[...] = jnp.sum(dpre, axis=0, keepdims=True).reshape(f).astype(_BF16)
        db2_s[...] = jnp.sum(dffn, axis=0, keepdims=True).reshape(d).astype(_BF16)
        weight_grad(dw1_s, _by_layer(n1, n3), dpre)
        weight_grad(dw2_s, _by_layer(a1, a3), dffn)
        weight_grad(dwq_s, _stack(n0, n2), _stack(dq0, dq2))
        weight_grad(dwo_s, _stack(o0, o2), _stack(dx1, dx3))

        def weight_writes(src, dst):
            _, rows, cols = src.shape
            c = min(cols, 2048)
            r = max(8, 16384 // c // 8 * 8)
            return [
                _tile_copy(src, dst, grad_sem, every, pl.ds(i, r), pl.ds(j, c))
                for i in range(0, rows, r)
                for j in range(0, cols, c)
            ]

        def grad_writes():
            whole = lambda src, dst: pltpu.make_async_copy(src, dst, grad_sem)
            return [
                [whole(out_s, out_hbm), whole(db1_s, db1_hbm)]
                + weight_writes(dwq_s, dwq_hbm)
                + weight_writes(dw1_s, dw1_hbm),
                [whole(dx_s, dx_hbm), whole(db2_s, db2_hbm)]
                + weight_writes(dwo_s, dwo_hbm)
                + weight_writes(dw2_s, dw2_hbm),
            ]

        _start(grad_writes())

        def by_batch(t):
            b = (_row(t.shape) // rep) % nb
            return jnp.concatenate(
                [jnp.where(b == i, t, 0.0) for i in range(nb)], axis=1
            ).astype(_BF16)

        @for_each_head
        def _(h):
            for key_ref, feat_ref, dst in ((ds_s, q_s, dk_s), (p_s, do_s, dv_s)):
                rhs = by_batch(feat_ref[h])
                for c in range(0, win, _KEY_CHUNK):
                    keys = slice(c, c + _KEY_CHUNK)
                    r = _dot(key_ref[h, :, keys], rhs, _TN).astype(_BF16)
                    dst[h, keys, :] = r[:, :dh]
                    dst[hkv + h, keys, :] = r[:, dh:]

        more_zeros(n_zero - zeros_issued[0])

        def window_writes(i):
            group = i // window_runs
            heads = pl.ds(group * _STREAMS, _STREAMS)
            r = pl.multiple_of((i - group * window_runs) * _WINDOW_RUN, _WINDOW_RUN)
            return [
                [
                    pltpu.make_async_copy(
                        src.at[heads, pl.ds(r, _WINDOW_RUN), :],
                        dst.at[heads, pl.ds(sk - win + r, _WINDOW_RUN), :],
                        window_sem,
                    )
                ]
                for src, dst in ((dk_s, dk_hbm), (dv_s, dv_hbm))
            ]

        zeros_per_window = n_zero // n_window

        @pl.loop(0, n_window)
        def _(i):
            _start(window_writes(i))
            for j in range(zeros_per_window):
                _wait(zero_writes(i * zeros_per_window + j))

        _wait(grad_writes())
        pl.loop(0, n_window)(lambda i: _wait(window_writes(i)))

    return kernel


@jax.jit
def pallas_interleave_layers__sliding_block_cached__dense_activation_gelu__decode_kernel(
    A_x: jax.Array,
    A_k_cache: jax.Array,
    A_v_cache: jax.Array,
    A_wq: jax.Array,
    A_wo: jax.Array,
    B_x: jax.Array,
    B_w1: jax.Array,
    B_b1: jax.Array,
    B_w2: jax.Array,
    B_b2: jax.Array,
    grad_out: jax.Array,
):
    del B_x
    nb, _, d = A_x.shape
    _, hkv, sk, dh = A_k_cache.shape
    rep = A_wq.shape[1] // (hkv * dh)
    f = B_w1.shape[1]
    win = min(4096, max(256, sk // 4))
    assert rep * dh == d

    def split_rows(w):
        return w.reshape(_STREAMS, w.shape[0] // _STREAMS, w.shape[1])

    inputs = (
        A_x.reshape(nb, d),
        grad_out.reshape(nb, d),
        A_k_cache.reshape(nb * hkv, sk, dh),
        A_v_cache.reshape(nb * hkv, sk, dh),
        split_rows(A_wq),
        split_rows(A_wo),
        split_rows(B_w1),
        B_b1,
        split_rows(B_w2),
        B_b2,
    )
    out_shape = [jax.ShapeDtypeStruct(a.shape, _BF16) for a in inputs]
    staging = [pltpu.VMEM(a.shape, _BF16) for a in inputs]
    staging[2] = staging[3] = pltpu.VMEM((nb * hkv, win, dh), _BF16)
    hbm = pl.BlockSpec(memory_space=pltpu.HBM)

    out, dx, dk, dv, dwq, dwo, dw1, db1, dw2, db2 = pl.pallas_call(
        _make_kernel(nb, hkv, rep, sk, win, dh, d, f),
        out_shape=out_shape,
        in_specs=[hbm] * len(inputs),
        out_specs=[hbm] * len(out_shape),
        scratch_shapes=staging + staging + [
            pltpu.VMEM((_STREAMS, _ZERO_RUN, dh), _BF16),
            pltpu.VMEM((hkv, 16, dh), _F32),
            pltpu.VMEM((hkv, 16, dh), _F32),
            pltpu.VMEM((hkv, 16, win), _F32),
            pltpu.VMEM((hkv, 16, win), _F32),
            pltpu.VMEM((4, hkv, 8, rep * dh), _F32),
            pltpu.SemaphoreType.DMA((5,)),
        ],
        compiler_params=pltpu.CompilerParams(vmem_limit_bytes=112 * 1024 * 1024),
    )(*inputs)
    return (
        out.reshape(A_x.shape),
        dx.reshape(A_x.shape),
        dk.reshape(A_k_cache.shape),
        dv.reshape(A_v_cache.shape),
        dwq.reshape(A_wq.shape),
        dwo.reshape(A_wo.shape),
        dw1.reshape(B_w1.shape),
        db1,
        dw2.reshape(B_w2.shape),
        db2,
    )
```
